```python
import jax
import jax.numpy as jnp

def _softmax(x, axis=-1):
    return jax.nn.softmax(x, axis=axis)

def _gelu(x):
    return jax.nn.gelu(x, approximate=True)

def _silu(x):
    return jax.nn.silu(x)

def _sigmoid(x):
    return jax.nn.sigmoid(x)

def _layernorm(x, axis=-1, eps=1e-05):
    m = jnp.mean(x, axis=axis, keepdims=True)
    v = jnp.var(x, axis=axis, keepdims=True)
    return (x - m) / jnp.sqrt(v + eps)

def _scatter_add(tgt, idx, src, axis=0):
    return tgt.at[idx].add(src)

def _segment_sum(src, seg, n):
    return jax.ops.segment_sum(src, seg, n)

class _Rng:

    def __init__(self, key):
        self._k = key

    def _next(self):
        self._k, sub = jax.random.split(self._k)
        return sub

    def normal(self, shape):
        return jax.random.normal(self._next(), shape, dtype=jnp.bfloat16)

    def randint(self, lo, hi, shape):
        return jax.random.randint(self._next(), shape, lo, hi, dtype=jnp.int32)

    def uniform(self, shape, lo=0.0, hi=1.0):
        return jax.random.uniform(self._next(), shape, jnp.bfloat16, lo, hi)

    def permutation(self, n):
        return jax.random.permutation(self._next(), n)
kernel_name = 'interleave_layers__sliding_local_dilated__mixer_gmlp__prompt'

def setup_inputs():
    _rng = _Rng(jax.random.key(int.from_bytes(__import__("os").urandom(4), "little")))
    _w = lambda a: (lambda t: t.astype(jnp.bfloat16) if jnp.issubdtype(t.dtype, jnp.floating) else t)(jnp.asarray(a))

    def _A_setup():
        B, S, D = (1, 2048, 576)
        return {'x': _w((lambda *s: _rng.normal(s) * 0.05)(B, S, D)), 'wqkv': _w((lambda *s: _rng.normal(s) * 0.05)(D, 3 * D)), 'wo': _w((lambda *s: _rng.normal(s) * 0.05)(D, D))}
    _A_in = _A_setup()

    def _B_setup():
        B, S, D, F = (1, 2048, 576, 4608)
        Fh = F // 2
        return {'x': _w((lambda *s: _rng.normal(s) * 0.05)(B, S, D)), 'w_in': _w((lambda *s: _rng.normal(s) * 0.05)(D, 2 * Fh)), 'w_sp': _w(0.01 * (lambda *s: _rng.normal(s) * 0.05)(S, S)), 'b_sp': _w(1.0 + 0.01 * (lambda *s: _rng.normal(s) * 0.05)(S)), 'w_out': _w((lambda *s: _rng.normal(s) * 0.05)(Fh, D))}
    _B_in = _B_setup()
    return {'A_x': _A_in['x'], 'A_wqkv': _A_in['wqkv'], 'A_wo': _A_in['wo'], 'B_x': _B_in['x'], 'B_w_in': _B_in['w_in'], 'B_w_sp': _B_in['w_sp'], 'B_b_sp': _B_in['b_sp'], 'B_w_out': _B_in['w_out']}

def reference(A_x, A_wqkv, A_wo, B_x, B_w_in, B_w_sp, B_b_sp, B_w_out):

    def _A_ref(x, wqkv, wo):
        B, S, D = x.shape
        H = 32
        Dh = D // H
        W, dil = (8, 2)
        qkv = (lambda x, *d: x.transpose(*d))((x @ wqkv).reshape(B, S, 3, H, Dh), 2, 0, 3, 1, 4)
        q, k, v = (qkv[0], qkv[1], qkv[2])
        scale = Dh ** (-0.5)
        pos = jnp.arange(S)
        off = jnp.arange(W) * dil
        idx = pos[:, None] - off[None, :]
        mask = idx >= 0
        idx_c = jnp.where(mask, idx, 0).reshape(-1)
        kg = k[:, :, idx_c, :].reshape(B, H, S, W, Dh)
        vg = v[:, :, idx_c, :].reshape(B, H, S, W, Dh)
        logits = jnp.einsum('bhsd,bhswd->bhsw', q, kg) * scale
        logits = jnp.where(mask[None, None, :, :], logits, -1000000000.0)
        attn = _softmax(logits, axis=-1)
        o = jnp.einsum('bhsw,bhswd->bhsd', attn, vg)
        return (lambda x, *d: x.transpose(*d))(o, 0, 2, 1, 3).reshape(B, S, D) @ wo

    def _B_ref(x, w_in, w_sp, b_sp, w_out):
        B, S, D = x.shape
        F = w_in.shape[-1]
        Fh = F // 2
        z = _gelu(jnp.einsum('bsd,df->bsf', x, w_in))
        z1 = z[..., :Fh].copy()
        z2 = _layernorm(z[..., Fh:], axis=-1)
        g = jnp.einsum('ts,bsf->btf', w_sp, z2) + b_sp[None, :, None]
        return jnp.einsum('bsf,fd->bsd', z1 * g, w_out)
    x = A_x
    x = x + _A_ref(_layernorm(x, axis=-1), A_wqkv, A_wo)
    x = x + _B_ref(_layernorm(x, axis=-1), B_w_in, B_w_sp, B_b_sp, B_w_out)
    x = x + _A_ref(_layernorm(x, axis=-1), A_wqkv, A_wo)
    x = x + _B_ref(_layernorm(x, axis=-1), B_w_in, B_w_sp, B_b_sp, B_w_out)
    return x
```

```python
import jax
import jax.numpy as jnp
from jax import lax
import jax.experimental.pallas as pl
import jax.experimental.pallas.tpu as pltpu

S, D, H, DH, FH = 2048, 576, 32, 18, 2304
TN = 256
HALO = 16
AR = 16
MC = 256
MG = 256
NA = 2
LC = 64
TK = 12
TQ = 64
MO = 192
PAT1 = 'abaaba' + 'baa' * 7 + 'baacccccc' + 'bcccccccc' + 'a' + ('b' + 'cccacccacc') * 7
PAT2 = 'abaab' + 'a' + 'baaaa' * 4 + 'ba' + 'b' + 'a' * 9
F32, BF16 = jnp.float32, jnp.bfloat16
NN = (((1,), (0,)), ((), ()))
NT = (((1,), (1,)), ((), ()))


def _dot(a, b, dims=NN):
    return lax.dot_general(a, b, dims, preferred_element_type=F32)


def _gelu(x):
    c = 0.7978845608028654
    return x * (0.5 + 0.5 * jnp.tanh(x * (c + (c * 0.044715) * (x * x))))


def _kernel(x_hbm, wqkv_hbm, wo_hbm, win_hbm, wsp_hbm, b_ref, wout_hbm, o_hbm,
            xb, xf, wqkv_raw, wo_raw, tmp, wqkv, wot, win, wint, wsp, wout, kb, vb, xn2, z1, z2, qb, ob, zt, hb, xn1, flag, sems):
    nt = S // TN
    xcp = [pltpu.make_async_copy(x_hbm.at[:, i * TN:(i + 1) * TN], xb.at[i], sems.at[8 + i]) for i in range(nt)]
    cps = [pltpu.make_async_copy(s, d, sems.at[i]) for i, (s, d) in enumerate([
        (wqkv_hbm, wqkv_raw), (wo_hbm, wo_raw), (win_hbm, win), (wsp_hbm, wsp), (wout_hbm, wout)])]
    cps[0].start()
    xcp[0].start()
    cps[1].start()
    xcp[1].start()
    kb[:, 0:HALO, :] = jnp.zeros((5, HALO, 128), F32)
    vb[:, 0:HALO, :] = jnp.zeros((5, HALO, 128), F32)
    cps[0].wait()
    cps[2].start()
    for i in range(2, nt):
        xcp[i].start()

    def rows(src, c):
        if c < 4:
            return src[c * 128:(c + 1) * 128, :].astype(F32)
        r = src[512:576, :].astype(F32)
        return jnp.concatenate([r, jnp.zeros_like(r)], axis=0)

    for c in range(5):
        r = rows(wqkv_raw, c)
        r = jnp.concatenate([r, jnp.zeros((128, 64), F32)], axis=1)
        tmp[c] = r.T
    for c in range(5):
        def ld(base, d):
            return tmp[c, pl.ds(base + d, H, stride=DH), :]
        blocks = []
        for base in (0, D, 2 * D):
            for t in range(4):
                blocks.append(jnp.concatenate([ld(base, 4 * t + u) for u in range(4)], axis=0))
        blocks.append(jnp.concatenate([ld(0, 16), ld(0, 17), ld(D, 16), ld(D, 17)], axis=0))
        blocks.append(jnp.concatenate([ld(2 * D, 16), ld(2 * D, 17), jnp.zeros((64, 128), F32)], axis=0))
        n = 128 if c < 4 else 64
        for t, blk in enumerate(blocks):
            wqkv[c * 128:c * 128 + n, t * 128:(t + 1) * 128] = blk.T[0:n].astype(BF16)
    cps[1].wait()
    xcp[0].wait()
    xcp[1].wait()
    w = wo_raw[...].astype(F32)
    w = jnp.concatenate([w, jnp.zeros((D, 64), F32)], axis=1)
    for c in range(5):
        tmp[c, 0:D, :] = w[:, c * 128:(c + 1) * 128]
    for c in range(5):
        n = 128 if c < 4 else 64
        for t in range(5):
            if t < 4:
                blk = jnp.concatenate([tmp[c, pl.ds(4 * t + u, H, stride=DH), :] for u in range(4)], axis=0)
            else:
                blk = jnp.concatenate([tmp[c, pl.ds(16 + u, H, stride=DH), :] for u in range(2)]
                                      + [jnp.zeros((64, 128), F32)], axis=0)
            wot[c * 128:c * 128 + n, t * 128:(t + 1) * 128] = blk.T[0:n].astype(BF16)
    scale = DH ** -0.5

    def tile0(i):
        return i * TN if isinstance(i, int) else pl.multiple_of(i * TN, TN)

    flag[0] = 0
    tok = [None, 0]

    def after(v, step=TK):
        if tok[0] is None:
            return v
        r = min(tok[1] // 8 * 8, tok[0].shape[0] // 2 - 8)
        tok[1] += step
        t = tok[0][r:r + 1, 0:v.shape[1]]
        return jnp.where(flag[0] != 0, jnp.broadcast_to(t, v.shape), v)

    def tsum(x):
        parts = [x[r:r + 8] for r in range(0, x.shape[0], 8)]
        while len(parts) > 1:
            parts = [parts[k] + parts[k + 1] if k + 1 < len(parts) else parts[k] for k in range(0, len(parts), 2)]
        return parts[0]

    def ln_rest(load, acc, n, ch, store):
        m = jnp.sum(acc, axis=0, keepdims=True) * (1.0 / n)
        acc = None
        for r in range(0, n, ch):
            d = load(r, ch) - after(m)
            p = tsum(d * d)
            acc = p if acc is None else acc + p
            yield
        rs = lax.rsqrt(jnp.sum(acc, axis=0, keepdims=True) * (1.0 / n) + 1e-5)
        for r in range(0, n, ch):
            store(r, ch, ((load(r, ch) - after(m)) * rs).astype(BF16))
            yield

    def stage_a(i, first=False):
        r0 = tile0(i)

        def ldx(r, n):
            return xb[i, r:r + n, :].astype(F32) if first else xf[i, r:r + n, :]

        def st1(r, n, v):
            xn1[r:r + n, :] = v

        yield from ln_rest(ldx, tsum(ldx(0, D)), D, D, st1)
        lane = lax.broadcasted_iota(jnp.int32, (TN, 128), 1)
        xn = xn1[...].T
        yield
        t = _dot(xn, wqkv[:, 1536:1792])
        qb[4] = jnp.where(lane < 64, t[:, 0:128] * scale, 0.0)
        kb[4, pl.ds(r0 + HALO, TN), :] = pltpu.roll(t[:, 0:128], 64, 1)
        vb[4, pl.ds(r0 + HALO, TN), :] = t[:, 128:256]
        t = _dot(xn, wqkv[:, 0:512])
        for j in range(4):
            qb[j] = t[:, j * 128:(j + 1) * 128] * scale
        t = _dot(xn, wqkv[:, 512:1024])
        for j in range(4):
            kb[j, pl.ds(r0 + HALO, TN), :] = t[:, j * 128:(j + 1) * 128]
        t = _dot(xn, wqkv[:, 1024:1536])
        for j in range(4):
            vb[j, pl.ds(r0 + HALO, TN), :] = t[:, j * 128:(j + 1) * 128]
        yield
        for c in range(TN // AR):
            q = [after(qb[j, c * AR:(c + 1) * AR, :], TQ if j == 4 else 0) for j in range(5)]
            ls = []
            for w in range(8):
                p = None
                for j in range(5):
                    kk = kb[j, pl.ds(r0 + HALO + c * AR - 2 * w, AR), :]
                    p = q[j] * kk if p is None else p + q[j] * kk
                p = p + pltpu.roll(p, 64, 1)
                p = p + pltpu.roll(p, 32, 1)
                if w > 0 and c * AR < 2 * w:
                    row = r0 + c * AR + lax.broadcasted_iota(jnp.int32, (AR, 128), 0)
                    p = jnp.where(row >= 2 * w, p, -1e9)
                ls.append(p)
            m = ls[0]
            for w in range(1, 8):
                m = jnp.maximum(m, ls[w])
            es = [jnp.exp(l - m) for l in ls]
            s = es[0]
            for w in range(1, 8):
                s = s + es[w]
            r = 1.0 / s
            for j in range(5):
                a = None
                for w in range(8):
                    vv = vb[j, pl.ds(r0 + HALO + c * AR - 2 * w, AR), :]
                    a = es[w] * vv if a is None else a + es[w] * vv
                ob[c * AR:(c + 1) * AR, j * 128:(j + 1) * 128] = (a * r).astype(BF16)
            yield
        acc = None
        for r in range(0, D, 192):
            x = ldx(r, 192) + _dot(wot[r:r + 192, :], ob[...], NT)
            xf[i, r:r + 192, :] = x
            acc = tsum(x) if acc is None else acc + tsum(x)
        yield

        def st2(r, n, v):
            xn2[i, r:r + n, :] = v

        yield from ln_rest(lambda r, n: xf[i, r:r + n, :], acc, D, 64, st2)

    def stage_b1(i, box):
        acc = None
        for c in range(FH // MC):
            zb = _dot(wint[FH + c * MC:FH + (c + 1) * MC, :], xn2[i])
            tok[:] = [zb, 0]
            zb = _gelu(zb)
            zt[c * MC:(c + 1) * MC, :] = zb
            acc = tsum(zb) if acc is None else acc + tsum(zb)
            box[0] = acc
            yield
        for c in range(FH // MC):
            za = _dot(wint[c * MC:(c + 1) * MC, :], xn2[i])
            tok[:] = [za, 0]
            za = _gelu(za)
            z1[i, c * MC:(c + 1) * MC, :] = za.astype(BF16)
            yield

    def stage_c(i, box):
        r0 = tile0(i)

        def st(r, n, v):
            z2[r:r + n, pl.ds(r0, TN)] = v

        yield from ln_rest(lambda r, n: zt[r:r + n, :], box[0], FH, LC, st)

    def stage_b2(i):
        r0 = tile0(i)
        for c in range(FH // MG):
            g = _dot(z2[c * MG:(c + 1) * MG, :], wsp[pl.ds(r0, TN), :], NT)
            tok[:] = [g, 0]
            g = g + b_ref[:, pl.ds(r0, TN)].astype(F32)
            hb[c * MG:(c + 1) * MG, :] = (z1[i, c * MG:(c + 1) * MG, :].astype(F32) * g).astype(BF16)
            yield
        for r in range(0, D, MO):
            x = xf[i, r:r + MO, :] + _dot(wout[r:r + MO, :], hb[...])
            xf[i, r:r + MO, :] = x
            xb[i, r:r + MO, :] = x.astype(BF16)

    def run(ga, gb, pattern, gc=iter(())):
        tok[0] = None
        for ch in pattern:
            next({'a': ga, 'b': gb, 'c': gc}[ch], None)
        for g in (gb, gc, ga):
            for _ in g:
                pass

    def phase1(ga, i):
        box = [None]
        run(ga, stage_b1(i, box), PAT1, stage_c(i, box))

    def transpose_win(c):
        c0 = pl.multiple_of(c * 1536, 128)
        wint[pl.ds(c0, 1536), :] = win[:, pl.ds(c0, 1536)].T

    def first_pass(i):
        @pl.when(i == 1)
        def _():
            cps[3].start()
            cps[4].start()
        phase1(stage_a(i + NA, True), i)

    def loop(lo, hi, f):
        lax.fori_loop(lo, hi, lambda i, _: f(i) or 0, 0)

    none = iter(())
    loop(0, NA, lambda i: run(stage_a(i, True), none, ''))
    cps[2].wait()
    for i in range(2, nt):
        xcp[i].wait()
    loop(0, 2 * FH // 1536, transpose_win)
    loop(0, nt - NA, first_pass)
    loop(nt - NA, nt, lambda i: phase1(none, i))
    cps[3].wait()
    cps[4].wait()
    loop(0, nt - 1, lambda i: run(none, stage_b2(i), ''))
    run(stage_a(0), stage_b2(nt - 1), PAT2)
    loop(0, nt - 1, lambda i: phase1(stage_a(i + 1), i))
    phase1(none, nt - 1)

    def last(i):
        run(none, stage_b2(i), '')
        pltpu.make_async_copy(xb.at[i], o_hbm.at[:, pl.ds(pl.multiple_of(i * TN, TN), TN)], sems.at[7]).start()

    loop(0, nt, last)
    for i in range(nt):
        pltpu.make_async_copy(xb.at[i], o_hbm.at[:, i * TN:(i + 1) * TN], sems.at[7]).wait()


@jax.jit
def pallas_interleave_layers__sliding_local_dilated__mixer_gmlp__prompt_kernel(
        A_x, A_wqkv, A_wo, B_x, B_w_in, B_w_sp, B_b_sp, B_w_out):
    nt = S // TN
    anyspec = pl.BlockSpec(memory_space=pl.ANY)
    out = pl.pallas_call(
        _kernel,
        out_shape=jax.ShapeDtypeStruct((D, S), BF16),
        in_specs=[anyspec, anyspec, anyspec, anyspec, anyspec, pl.BlockSpec(memory_space=pltpu.VMEM), anyspec],
        out_specs=anyspec,
        scratch_shapes=[
            pltpu.VMEM((nt, D, TN), BF16), pltpu.VMEM((nt, D, TN), F32),
            pltpu.VMEM((D, 3 * D), BF16), pltpu.VMEM((D, D), BF16), pltpu.VMEM((5, 1792, 128), F32),
            pltpu.VMEM((D, 1792), BF16), pltpu.VMEM((D, 640), BF16),
            pltpu.VMEM((D, 2 * FH), BF16), pltpu.VMEM((2 * FH, D), BF16),
            pltpu.VMEM((S, S), BF16), pltpu.VMEM((D, FH), BF16),
            pltpu.VMEM((5, S + HALO, 128), F32), pltpu.VMEM((5, S + HALO, 128), F32),
            pltpu.VMEM((nt, D, TN), BF16),
            pltpu.VMEM((nt, FH, TN), BF16), pltpu.VMEM((FH, S), BF16),
            pltpu.VMEM((5, TN, 128), F32), pltpu.VMEM((TN, 640), BF16), pltpu.VMEM((FH, TN), F32), pltpu.VMEM((FH, TN), BF16),
            pltpu.VMEM((D, TN), BF16),
            pltpu.SMEM((1,), jnp.int32),
            pltpu.SemaphoreType.DMA((8 + nt,)),
        ],
        compiler_params=pltpu.CompilerParams(vmem_limit_bytes=110 * 1024 * 1024),
    )(A_x.reshape(S, D).T, A_wqkv, A_wo, B_w_in, B_w_sp, B_b_sp.reshape(1, S), B_w_out.T)
    return out.T.reshape(1, S, D)
```
